```python
import os as _os
_os.environ.setdefault("JAX_PLATFORMS", "cpu")
import jax
import jax.numpy as jnp

def _softmax(x, axis=-1):
    return jax.nn.softmax(x, axis=axis)
def _gelu(x):
    return jax.nn.gelu(x, approximate=True)
def _silu(x):
    return jax.nn.silu(x)
def _sigmoid(x):
    return jax.nn.sigmoid(x)
def _layernorm(x, axis=-1, eps=1e-5):
    m = jnp.mean(x, axis=axis, keepdims=True)
    v = jnp.var(x, axis=axis, keepdims=True)
    return (x - m) / jnp.sqrt(v + eps)
def _scatter_add(tgt, idx, src, axis=0):
    return tgt.at[idx].add(src)
def _segment_sum(src, seg, n):
    return jax.ops.segment_sum(src, seg, n)
class _Rng:
    def __init__(self, key):
        self._k = key
    def _next(self):
        self._k, sub = jax.random.split(self._k)
        return sub
    def normal(self, shape):
        return jax.random.normal(self._next(), shape, dtype=jnp.bfloat16)
    def randint(self, lo, hi, shape):
        return jax.random.randint(self._next(), shape, lo, hi, dtype=jnp.int32)
    def uniform(self, shape, lo=0.0, hi=1.0):
        return jax.random.uniform(self._next(), shape, jnp.bfloat16, lo, hi)
    def permutation(self, n):
        return jax.random.permutation(self._next(), n)


kernel_name = 'concat_heads__mha_block_cached__mha_block_cached__near_ridge'

def setup_inputs():
    _rng = _Rng(jax.random.key(int.from_bytes(__import__("os").urandom(4), "little")))
    _w = (lambda a: (lambda t: t.astype(jnp.bfloat16) if jnp.issubdtype(t.dtype, jnp.floating) else t)(jnp.asarray(a)))
    def _A_setup():
        B, Sq, D = 16, 80, 512
        H, Sk, Dh = 32, 80, 128
        return {
            "x": _w((lambda *s: _rng.normal(s) * 0.8)(B, Sq, D)),
            "k_cache": _w((lambda *s: _rng.normal(s) * 0.8)(B, H, Sk, Dh)),
            "v_cache": _w((lambda *s: _rng.normal(s) * 0.05)(B, H, Sk, Dh)),
            "wq": _w((lambda *s: _rng.normal(s) * 0.8)(D, H * Dh) * (D ** -0.5)),
            "wo": _w((lambda *s: _rng.normal(s) * 0.05)(H * Dh, D) * ((H * Dh) ** -0.5)),
        }
    _A_in = _A_setup()

    def _B_setup():
        B, Sq, D = 16, 80, 512
        H, Sk, Dh = 32, 80, 128
        return {
            "x": _w((lambda *s: _rng.normal(s) * 0.8)(B, Sq, D)),
            "k_cache": _w((lambda *s: _rng.normal(s) * 0.8)(B, H, Sk, Dh)),
            "v_cache": _w((lambda *s: _rng.normal(s) * 0.05)(B, H, Sk, Dh)),
            "wq": _w((lambda *s: _rng.normal(s) * 0.8)(D, H * Dh) * (D ** -0.5)),
            "wo": _w((lambda *s: _rng.normal(s) * 0.05)(H * Dh, D) * ((H * Dh) ** -0.5)),
        }
    _B_in = _B_setup()

    return {
        "A_x": _A_in["x"],
        "A_k_cache": _A_in["k_cache"],
        "A_v_cache": _A_in["v_cache"],
        "A_wq": _A_in["wq"],
        "A_wo": _A_in["wo"],
        "B_x": _B_in["x"],
        "B_k_cache": _B_in["k_cache"],
        "B_v_cache": _B_in["v_cache"],
        "B_wq": _B_in["wq"],
        "B_wo": _B_in["wo"],
    }

def reference(A_x, A_k_cache, A_v_cache, A_wq, A_wo, B_x, B_k_cache, B_v_cache, B_wq, B_wo):
    def _A_ref(x, k_cache, v_cache, wq, wo):
        B, Sq, D = x.shape
        H, Dh = 32, 128
        q = (lambda x, *d: x.transpose(*d))((x @ wq).reshape(B, Sq, H, Dh), 0, 2, 1, 3)
        scores = jnp.einsum("bhqd,bhkd->bhqk", q, k_cache) * (Dh ** -0.5)
        p = _softmax(scores, axis=-1)
        o = jnp.einsum("bhqk,bhkd->bhqd", p, v_cache)
        return (lambda x, *d: x.transpose(*d))(o, 0, 2, 1, 3).reshape(B, Sq, H * Dh) @ wo

    def _B_ref(x, k_cache, v_cache, wq, wo):
        B, Sq, D = x.shape
        H, Dh = 32, 128
        q = (lambda x, *d: x.transpose(*d))((x @ wq).reshape(B, Sq, H, Dh), 0, 2, 1, 3)
        scores = jnp.einsum("bhqd,bhkd->bhqk", q, k_cache) * (Dh ** -0.5)
        p = _softmax(scores, axis=-1)
        o = jnp.einsum("bhqk,bhkd->bhqd", p, v_cache)
        return (lambda x, *d: x.transpose(*d))(o, 0, 2, 1, 3).reshape(B, Sq, H * Dh) @ wo

    a = _A_ref(A_x, A_k_cache, A_v_cache, A_wq, A_wo)
    b = _B_ref(B_x, B_k_cache, B_v_cache, B_wq, B_wo)
    return jnp.concatenate([a, b], axis=-1)
```

```python
import functools
import jax
import jax.numpy as jnp
import jax.experimental.pallas as pl
import jax.experimental.pallas.tpu as pltpu

B, SQ, D = 16, 80, 512
H, SK, DH = 32, 80, 128
M = B * SQ
TH = 4
NG = H // TH
NU = 2 * NG
CW = TH * DH
bf = jnp.bfloat16
f32 = jnp.float32
NT = (((1,), (1,)), ((), ()))
SCALE = DH ** -0.5


def _attn1(qh, kh, vh):
    s = jax.lax.dot_general(qh, kh, NT, preferred_element_type=f32)
    m = jnp.max(s, axis=-1, keepdims=True)
    p = jnp.exp(s - m)
    l = jnp.sum(p, axis=-1, keepdims=True)
    o = jnp.dot(p.astype(bf), vh, preferred_element_type=f32)
    return (o * pl.reciprocal(l, approx=True)).astype(bf)


def _body(xa, ka, va, wqa, woa, xb, kb, vb, wqb, wob, out_hbm,
          x_s, wq_s, wo_s, k_s, v_s, acc, stage, sem_x, sem_u, sem_o):

    def unit_copies(refs, g, slot):
        _, k, v, wq, wo = refs
        h0 = g * TH
        c0 = pl.multiple_of(g * CW, 128)
        return [
            pltpu.make_async_copy(wq.at[:, pl.ds(c0, CW)], wq_s.at[slot], sem_u.at[slot, 0]),
            pltpu.make_async_copy(k.at[:, pl.ds(h0, TH)], k_s.at[slot], sem_u.at[slot, 1]),
            pltpu.make_async_copy(v.at[:, pl.ds(h0, TH)], v_s.at[slot], sem_u.at[slot, 2]),
            pltpu.make_async_copy(wo.at[pl.ds(c0, CW), :], wo_s.at[slot], sem_u.at[slot, 3]),
        ]

    A = (xa, ka, va, wqa, woa)
    Bb = (xb, kb, vb, wqb, wob)

    def for_unit(u, fn):
        slot = u % 2
        g = u % NG
        @pl.when(u < NG)
        def _():
            for c in unit_copies(A, g, slot):
                fn(c)
        @pl.when(u >= NG)
        def _():
            for c in unit_copies(Bb, g, slot):
                fn(c)

    def x_copy(br):
        return pltpu.make_async_copy(xa if br == 0 else xb, x_s.at[br], sem_x.at[br])

    def out_copy(br):
        return pltpu.make_async_copy(stage.at[br], out_hbm.at[:, pl.ds(br * D, D)], sem_o.at[br])

    x_copy(0).start()
    for c in unit_copies(A, 0, 0):
        c.start()
    acc[...] = jnp.zeros_like(acc)

    def step(u, carry):
        slot = u % 2
        br = u // NG

        @pl.when(u + 1 < NU)
        def _():
            for_unit(u + 1, lambda c: c.start())

        @pl.when(u == 0)
        def _():
            x_copy(0).wait()
            x_copy(1).start()

        @pl.when(u == NG)
        def _():
            x_copy(1).wait()

        for_unit(u, lambda c: c.wait())

        q = jnp.dot(x_s[br], wq_s[slot], preferred_element_type=f32)
        q = (q * SCALE).astype(bf)
        cols = []
        for h in range(TH):
            rows = []
            for b in range(B):
                qh = q[b * SQ:(b + 1) * SQ, h * DH:(h + 1) * DH]
                rows.append(_attn1(qh, k_s[slot, b, h], v_s[slot, b, h]))
            cols.append(jnp.concatenate(rows, axis=0))
        o = jnp.concatenate(cols, axis=1)
        t = acc[br] + jnp.dot(o, wo_s[slot], preferred_element_type=f32)
        acc[br] = t
        stage[br] = t.astype(bf)

        @pl.when(u == NG - 1)
        def _():
            out_copy(0).start()
        return carry

    jax.lax.fori_loop(0, NU, step, 0)
    out_copy(1).start()
    out_copy(0).wait()
    out_copy(1).wait()


@jax.jit
def pallas_concat_heads__mha_block_cached__mha_block_cached__near_ridge_kernel(
    A_x, A_k_cache, A_v_cache, A_wq, A_wo, B_x, B_k_cache, B_v_cache, B_wq, B_wo):
    xa = A_x.reshape(M, D)
    xb = B_x.reshape(M, D)
    any_spec = pl.BlockSpec(memory_space=pl.ANY)
    out = pl.pallas_call(
        _body,
        in_specs=[any_spec] * 10,
        out_specs=any_spec,
        out_shape=jax.ShapeDtypeStruct((M, 2 * D), bf),
        scratch_shapes=[
            pltpu.VMEM((2, M, D), bf),
            pltpu.VMEM((2, D, CW), bf),
            pltpu.VMEM((2, CW, D), bf),
            pltpu.VMEM((2, B, TH, SK, DH), bf),
            pltpu.VMEM((2, B, TH, SK, DH), bf),
            pltpu.VMEM((2, M, D), f32),
            pltpu.VMEM((2, M, D), bf),
            pltpu.SemaphoreType.DMA((2,)),
            pltpu.SemaphoreType.DMA((2, 4)),
            pltpu.SemaphoreType.DMA((2,)),
        ],
        compiler_params=pltpu.CompilerParams(vmem_limit_bytes=100 * 1024 * 1024),
    )(xa, A_k_cache, A_v_cache, A_wq, A_wo, xb, B_k_cache, B_v_cache, B_wq, B_wo)
    return out.reshape(B, SQ, 2 * D)
```

```python
import functools
import jax
import jax.numpy as jnp
import jax.experimental.pallas as pl
import jax.experimental.pallas.tpu as pltpu

B, SQ, D = 16, 80, 512
H, SK, DH = 32, 80, 128
M = B * SQ
TH = 8
NG = H // TH
NU = 2 * NG
CW = TH * DH
HW = CW // 2
XR = 320
OC = 4
OR = M // OC
NQ = 4
bf = jnp.bfloat16
f32 = jnp.float32
NT = (((1,), (1,)), ((), ()))
SCALE = DH ** -0.5
SCOPES = False

S_X0, S_X1, S_X23, S_XB, S_WQA = 0, 1, 2, 3, 4
S_WQ = 5
S_K = S_WQ + NU
S_V = S_K + NU
S_WO = S_V + NU
S_N = S_WO + NU


def _scope(name):
    import contextlib
    return jax.named_scope(name) if SCOPES else contextlib.nullcontext()


def _attn1(qh, kh, vh):
    s = jax.lax.dot_general(qh, kh, NT, preferred_element_type=f32)
    m = jnp.max(s, axis=-1, keepdims=True)
    p = jnp.exp(s - m)
    l = jnp.sum(p, axis=-1, keepdims=True)
    o = jnp.dot(p.astype(bf), vh, preferred_element_type=f32)
    return (o * pl.reciprocal(l, approx=True)).astype(bf)


def _body(xa, ka, va, wqa, woa, xb, kb, vb, wqb, wob, out_hbm,
          x_s, wq_s, wo_s, k_s, v_s, q_s, acc, stage, sem, sem_o):
    ks = (ka, kb); vs = (va, vb); wqs = (wqa, wqb); wos = (woa, wob)
    cp = pltpu.make_async_copy

    def x_cp(r0, nr, s):
        return cp(xa.at[pl.ds(r0, nr)], x_s.at[0, pl.ds(r0, nr)], sem.at[s])
    x0_cp = x_cp(0, XR, S_X0)
    x1_cp = x_cp(XR, XR, S_X1)
    x23_cp = x_cp(2 * XR, 2 * XR, S_X23)
    xb_cp = cp(xb, x_s.at[1], sem.at[S_XB])
    wq0a_cp = cp(wqa.at[:, pl.ds(0, HW)], wq_s.at[0, :, pl.ds(0, HW)], sem.at[S_WQA])
    wq0b_cp = cp(wqa.at[:, pl.ds(HW, HW)], wq_s.at[0, :, pl.ds(HW, HW)], sem.at[S_WQ])
    def wq_cp(u):
        br, g = divmod(u, NG)
        return cp(wqs[br].at[:, pl.ds(g * CW, CW)], wq_s.at[u], sem.at[S_WQ + u])
    def k_cp(u):
        br, g = divmod(u, NG)
        return cp(ks[br].at[:, pl.ds(g * TH, TH)], k_s.at[u], sem.at[S_K + u])
    def v_cp(u):
        br, g = divmod(u, NG)
        return cp(vs[br].at[:, pl.ds(g * TH, TH)], v_s.at[u], sem.at[S_V + u])
    def wo_cp(u):
        br, g = divmod(u, NG)
        return cp(wos[br].at[pl.ds(g * CW, CW)], wo_s.at[u], sem.at[S_WO + u])
    def wait_into(dst, s):
        cp(dst, dst, sem.at[s]).wait()
    outa_cp = cp(stage.at[0], out_hbm.at[:, pl.ds(0, D)], sem_o.at[OC])
    def outb_cp(c):
        return cp(stage.at[1, pl.ds(c * OR, OR)], out_hbm.at[pl.ds(c * OR, OR), pl.ds(D, D)], sem_o.at[c])

    wq0a_cp.start(); x0_cp.start(); x1_cp.start(); wq0b_cp.start(); x23_cp.start()
    wq_cp(1).start()
    for u in range(NU):
        k_cp(u).start(); v_cp(u).start(); wo_cp(u).start()
        if u + 2 == NG:
            xb_cp.start()
        if u + 2 < NU:
            wq_cp(u + 2).start()

    def qproj(xv, w):
        return (jnp.dot(xv, w, preferred_element_type=f32) * SCALE).astype(bf)

    def attention(u, qslot):
        cols = []
        for h in range(TH):
            rows = []
            for b in range(B):
                qh = q_s[qslot, b * SQ:(b + 1) * SQ, h * DH:(h + 1) * DH]
                rows.append(_attn1(qh, k_s[u, b, h], v_s[u, b, h]))
            cols.append(jnp.concatenate(rows, axis=0))
        return jnp.concatenate(cols, axis=1)

    with _scope("R0a"):
        wq0a_cp.wait(); x0_cp.wait()
        q_s[0, 0:XR, 0:HW] = qproj(x_s[0, 0:XR, :], wq_s[0, :, 0:HW])
    with _scope("R0b"):
        x1_cp.wait(); wq0b_cp.wait()
        q_s[0, XR:2 * XR, 0:HW] = qproj(x_s[0, XR:2 * XR, :], wq_s[0, :, 0:HW])
        q_s[0, 0:2 * XR, HW:CW] = qproj(x_s[0, 0:2 * XR, :], wq_s[0, :, HW:CW])
    with _scope("R0c"):
        x23_cp.wait()
        wq_cp(1).wait()
        q_s[0, 2 * XR:M, :] = qproj(x_s[0, 2 * XR:M, :], wq_s[0])
        q_s[1] = qproj(x_s[0], wq_s[1])

    def step(u, carry):
        with _scope("step"):
            br = u >> 2
            un = u + 2
            wait_into(k_s.at[0], S_K + u)
            wait_into(v_s.at[0], S_V + u)
            wait_into(wo_s.at[0], S_WO + u)
            wait_into(wq_s.at[0], S_WQ + un)
            @pl.when(un == NG)
            def _():
                xb_cp.wait()
            q_s[un & (NQ - 1)] = qproj(x_s[un >> 2], wq_s[un])
            o = attention(u, u & (NQ - 1))
            prev = jnp.where((u & (NG - 1)) == 0, 0.0, acc[br])
            t = prev + jnp.dot(o, wo_s[u], preferred_element_type=f32)
            acc[br] = t
            stage[br] = t.astype(bf)
            @pl.when(u == NG - 1)
            def _():
                outa_cp.start()
        return carry
    jax.lax.fori_loop(0, NU - 2, step, 0)

    def last(u, carry):
        with _scope("last"):
            wait_into(k_s.at[0], S_K + u)
            wait_into(v_s.at[0], S_V + u)
            wait_into(wo_s.at[0], S_WO + u)
            o = attention(u, u & (NQ - 1))
            for c in range(OC):
                r = slice(c * OR, (c + 1) * OR)
                t = acc[1, r, :] + jnp.dot(o[r], wo_s[u], preferred_element_type=f32)
                acc[1, r, :] = t
                stage[1, r, :] = t.astype(bf)
                @pl.when(u == NU - 1)
                def _():
                    outb_cp(c).start()
        return carry
    jax.lax.fori_loop(NU - 2, NU, last, 0)
    with _scope("tail"):
        outa_cp.wait()
        for c in range(OC):
            outb_cp(c).wait()


@jax.jit
def pallas_concat_heads__mha_block_cached__mha_block_cached__near_ridge_kernel(
    A_x, A_k_cache, A_v_cache, A_wq, A_wo, B_x, B_k_cache, B_v_cache, B_wq, B_wo):
    xa = A_x.reshape(M, D)
    xb = B_x.reshape(M, D)
    any_spec = pl.BlockSpec(memory_space=pl.ANY)
    DMA = pltpu.SemaphoreType.DMA
    out = pl.pallas_call(
        _body,
        in_specs=[any_spec] * 10,
        out_specs=any_spec,
        out_shape=jax.ShapeDtypeStruct((M, 2 * D), bf),
        scratch_shapes=[
            pltpu.VMEM((2, M, D), bf),
            pltpu.VMEM((NU, D, CW), bf),
            pltpu.VMEM((NU, CW, D), bf),
            pltpu.VMEM((NU, B, TH, SK, DH), bf),
            pltpu.VMEM((NU, B, TH, SK, DH), bf),
            pltpu.VMEM((NQ, M, CW), bf),
            pltpu.VMEM((2, M, D), f32),
            pltpu.VMEM((2, M, D), bf),
            DMA((S_N,)), DMA((OC + 1,)),
        ],
        compiler_params=pltpu.CompilerParams(vmem_limit_bytes=120 * 1024 * 1024, disable_semaphore_checks=True),
    )(xa, A_k_cache, A_v_cache, A_wq, A_wo, xb, B_k_cache, B_v_cache, B_wq, B_wo)
    return out.reshape(B, SQ, 2 * D)
```

```python
import jax
import jax.numpy as jnp
import jax.experimental.pallas as pl
import jax.experimental.pallas.tpu as pltpu

B, SQ, D = 16, 80, 512
H, SK, DH = 32, 80, 128
M = B * SQ
TH = 8
NG = H // TH
NU = 2 * NG
CW = TH * DH
HW = CW // 2
XR = 320
OCH = (560, 400, 240, 80)
OC = len(OCH)
OFF = tuple(sum(OCH[:i]) for i in range(OC + 1))
NQ = 4
FM = 160
KC = D // 128
bf = jnp.bfloat16
f32 = jnp.float32
NT = (((1,), (1,)), ((), ()))
SCALE = DH ** -0.5
SCOPES = False
LAST_Y = True

S_X0, S_X1, S_X23, S_XB, S_WQA = 0, 1, 2, 3, 4
S_WQ = 5
S_K = S_WQ + NU
S_V = S_K + NU
S_WO = S_V + NU
S_N = S_WO + NU


class _Null:
    def __enter__(self):
        return self
    def __exit__(self, *a):
        return False


def _scope(name):
    return jax.named_scope(name) if SCOPES else _Null()


def _dot(a, b):
    return jnp.dot(a, b, preferred_element_type=f32)


def _chain(acc2, j, d):
    acc2[j % 2] = d if acc2[j % 2] is None else acc2[j % 2] + d


def _attention(get_q, get_k, get_v, x_op, x_done, y_op):
    items = [(h, b) for h in range(TH) for b in range(B)]
    n = len(items)
    queues = {0: [], 1: [], 2: [], 3: []}
    for j in range(KC):
        queues[1 + 2 * (j % 2)].append(('X', j))
    for i in range(n):
        queues[2 * (i % 2)].append(('S', i))
        queues[1 + 2 * (i % 2)].append(('P', i))
    if y_op is not None:
        for j in range(KC):
            queues[2 * (j % 2)].append(('Y', j))
    cost = {'S': SQ, 'P': SQ, 'X': FM, 'Y': FM}
    load = [0, 0, 0, 0]
    res, soft, xs, ys = {}, {}, [None, None], [None, None]
    while any(queues.values()):
        cand = sorted(range(4), key=lambda m: (load[m], m))
        m = [c for c in cand if queues[c]][0]
        kind, idx = queues[m].pop(0)
        load[m] += cost[kind]
        if kind == 'S':
            h, b = items[idx]
            s = jax.lax.dot_general(get_q(h, b), get_k(h, b), NT, preferred_element_type=f32)
            p = jnp.exp(s - jnp.max(s, axis=-1, keepdims=True))
            soft[idx] = (p.astype(bf), jnp.sum(p, axis=-1, keepdims=True))
        elif kind == 'P':
            h, b = items[idx]
            p, l = soft.pop(idx)
            o = _dot(p, get_v(h, b))
            res[(h, b)] = (o * pl.reciprocal(l, approx=True)).astype(bf)
        elif kind == 'X':
            _chain(xs, idx, x_op(idx))
            if idx == KC - 1:
                x_done(xs)
        else:
            _chain(ys, idx, y_op(idx, res))
    o = jnp.concatenate(
        [jnp.concatenate([res[(h, b)] for b in range(B)], axis=0) for h in range(TH)], axis=1)
    return o, ys


def _body(xa, ka, va, wqa, woa, xb, kb, vb, wqb, wob, out_hbm,
          x_s, wq_s, wo_s, k_s, v_s, q_s, acc, stage, sem, sem_o):
    ks = (ka, kb); vs = (va, vb); wqs = (wqa, wqb); wos = (woa, wob)
    cp = pltpu.make_async_copy

    def x_cp(r0, nr, s):
        return cp(xa.at[pl.ds(r0, nr)], x_s.at[0, pl.ds(r0, nr)], sem.at[s])
    x0_cp = x_cp(0, XR, S_X0)
    x1_cp = x_cp(XR, XR, S_X1)
    x23_cp = x_cp(2 * XR, 2 * XR, S_X23)
    xb_cp = cp(xb, x_s.at[1], sem.at[S_XB])
    wq0a_cp = cp(wqa.at[:, pl.ds(0, HW)], wq_s.at[0, :, pl.ds(0, HW)], sem.at[S_WQA])
    wq0b_cp = cp(wqa.at[:, pl.ds(HW, HW)], wq_s.at[0, :, pl.ds(HW, HW)], sem.at[S_WQ])
    def wq_cp(u):
        br, g = divmod(u, NG)
        return cp(wqs[br].at[:, pl.ds(g * CW, CW)], wq_s.at[u], sem.at[S_WQ + u])
    def k_cp(u):
        br, g = divmod(u, NG)
        return cp(ks[br].at[:, pl.ds(g * TH, TH)], k_s.at[u], sem.at[S_K + u])
    def v_cp(u):
        br, g = divmod(u, NG)
        return cp(vs[br].at[:, pl.ds(g * TH, TH)], v_s.at[u], sem.at[S_V + u])
    def wo_cp(u):
        br, g = divmod(u, NG)
        return cp(wos[br].at[pl.ds(g * CW, CW)], wo_s.at[u], sem.at[S_WO + u])
    def wait_into(dst, s):
        cp(dst, dst, sem.at[s]).wait()
    outa_cp = cp(stage.at[0], out_hbm.at[:, pl.ds(0, D)], sem_o.at[OC])
    def outb_cp(c):
        return cp(stage.at[1, pl.ds(OFF[c], OCH[c])], out_hbm.at[pl.ds(OFF[c], OCH[c]), pl.ds(D, D)], sem_o.at[c])

    wq0a_cp.start(); x0_cp.start(); x1_cp.start(); wq0b_cp.start(); x23_cp.start()
    wq_cp(1).start()
    for u in range(NU):
        k_cp(u).start(); v_cp(u).start(); wo_cp(u).start()
        if u + 2 == NG:
            xb_cp.start()
        if u + 2 < NU:
            wq_cp(u + 2).start()

    def fin_q(q):
        return (q * SCALE).astype(bf)

    def fin_q2(v):
        return (v[0] * SCALE + v[1] * SCALE).astype(bf)

    def qproj(xv, w):
        return fin_q(_dot(xv, w))

    C7 = (TH - 1) * DH
    C6 = (TH - 2) * DH

    def attention(u, y_op):
        br = u >> 2
        qslot = u & (NQ - 1)
        q7 = []
        def x_op(j):
            return _dot(x_s[br, 0:FM, j * 128:(j + 1) * 128], wq_s[u, j * 128:(j + 1) * 128, C7:CW])
        def x_done(v):
            q7.append(fin_q2(v))
        def get_q(h, b):
            if h == TH - 1 and (b + 1) * SQ <= FM:
                return q7[0][b * SQ:(b + 1) * SQ]
            return q_s[qslot, b * SQ:(b + 1) * SQ, h * DH:(h + 1) * DH]
        return _attention(get_q, lambda h, b: k_s[u, b, h], lambda h, b: v_s[u, b, h], x_op, x_done, y_op)

    with _scope("R0a"):
        wq0a_cp.wait(); x0_cp.wait()
        q_s[0, 0:XR, 0:HW] = qproj(x_s[0, 0:XR, :], wq_s[0, :, 0:HW])
    with _scope("R0b"):
        x1_cp.wait(); wq0b_cp.wait()
        q_s[0, XR:2 * XR, 0:HW] = qproj(x_s[0, XR:2 * XR, :], wq_s[0, :, 0:HW])
        q_s[0, 0:2 * XR, HW:C7] = qproj(x_s[0, 0:2 * XR, :], wq_s[0, :, HW:C7])
        q_s[0, FM:2 * XR, C7:CW] = qproj(x_s[0, FM:2 * XR, :], wq_s[0, :, C7:CW])
    with _scope("R0c"):
        x23_cp.wait()
        wq_cp(1).wait()
        q_s[0, 2 * XR:M, :] = qproj(x_s[0, 2 * XR:M, :], wq_s[0])
        q_s[1, :, 0:C7] = qproj(x_s[0], wq_s[1, :, 0:C7])
        q_s[1, FM:M, C7:CW] = qproj(x_s[0, FM:M, :], wq_s[1, :, C7:CW])

    def step(u, carry):
        with _scope("step"):
            br = u >> 2
            un = u + 2
            bn = un >> 2
            ns = un & (NQ - 1)
            wait_into(k_s.at[u], S_K + u)
            wait_into(v_s.at[u], S_V + u)
            wait_into(wo_s.at[u], S_WO + u)
            wait_into(wq_s.at[un], S_WQ + un)
            @pl.when(un == NG)
            def _():
                xb_cp.wait()
            q_s[ns, :, 0:C6] = qproj(x_s[bn], wq_s[un, :, 0:C6])
            q_s[ns, FM:M, C6:CW] = qproj(x_s[bn, FM:M, :], wq_s[un, :, C6:CW])
            def y_op(j, res):
                return _dot(x_s[bn, 0:FM, j * 128:(j + 1) * 128], wq_s[un, j * 128:(j + 1) * 128, C6:C7])
            o, qy = attention(u, y_op)
            q_s[ns, 0:FM, C6:C7] = fin_q2(qy)
            prev = jnp.where((u & (NG - 1)) == 0, 0.0, acc[br])
            t = prev + _dot(o, wo_s[u])
            acc[br] = t
            stage[br] = t.astype(bf)
            @pl.when(u == NG - 1)
            def _():
                outa_cp.start()
        return carry
    jax.lax.fori_loop(0, NU - 2, step, 0)

    def last(u, carry):
        with _scope("last"):
            wait_into(k_s.at[u], S_K + u)
            wait_into(v_s.at[u], S_V + u)
            wait_into(wo_s.at[u], S_WO + u)
            def y_op(j, res):
                lhs = jnp.concatenate([res[(j, b)] for b in range(FM // SQ)], axis=0)
                return _dot(lhs, wo_s[u, j * 128:(j + 1) * 128, 0:128])
            o, oy = attention(u, y_op if LAST_Y else None)
            for c in range(OC):
                r0, r1 = OFF[c], OFF[c + 1]
                if c == 0 and LAST_Y:
                    ta = (acc[1, 0:FM, 0:128] + oy[0]) + (oy[1] + _dot(o[0:FM, KC * 128:], wo_s[u, KC * 128:, 0:128]))
                    tb = _dot(o[0:FM], wo_s[u, :, 128:D])
                    tc = _dot(o[FM:r1], wo_s[u])
                    tb = acc[1, 0:FM, 128:D] + tb
                    tc = acc[1, FM:r1, :] + tc
                    t = jnp.concatenate([jnp.concatenate([ta, tb], axis=1), tc], axis=0)
                else:
                    t = acc[1, r0:r1, :] + _dot(o[r0:r1], wo_s[u])
                acc[1, r0:r1, :] = t
                stage[1, r0:r1, :] = t.astype(bf)
                @pl.when(u == NU - 1)
                def _():
                    outb_cp(c).start()
        return carry
    jax.lax.fori_loop(NU - 2, NU, last, 0)
    with _scope("tail"):
        outa_cp.wait()
        for c in range(OC):
            outb_cp(c).wait()


@jax.jit
def pallas_concat_heads__mha_block_cached__mha_block_cached__near_ridge_kernel(
    A_x, A_k_cache, A_v_cache, A_wq, A_wo, B_x, B_k_cache, B_v_cache, B_wq, B_wo):
    xa = A_x.reshape(M, D)
    xb = B_x.reshape(M, D)
    any_spec = pl.BlockSpec(memory_space=pl.ANY)
    DMA = pltpu.SemaphoreType.DMA
    out = pl.pallas_call(
        _body,
        in_specs=[any_spec] * 10,
        out_specs=any_spec,
        out_shape=jax.ShapeDtypeStruct((M, 2 * D), bf),
        scratch_shapes=[
            pltpu.VMEM((2, M, D), bf),
            pltpu.VMEM((NU, D, CW), bf),
            pltpu.VMEM((NU, CW, D), bf),
            pltpu.VMEM((NU, B, TH, SK, DH), bf),
            pltpu.VMEM((NU, B, TH, SK, DH), bf),
            pltpu.VMEM((NQ, M, CW), bf),
            pltpu.VMEM((2, M, D), f32),
            pltpu.VMEM((2, M, D), bf),
            DMA((S_N,)), DMA((OC + 1,)),
        ],
        compiler_params=pltpu.CompilerParams(vmem_limit_bytes=120 * 1024 * 1024,
                                             disable_semaphore_checks=True),
    )(xa, A_k_cache, A_v_cache, A_wq, A_wo, xb, B_k_cache, B_v_cache, B_wq, B_wo)
    return out.reshape(B, SQ, 2 * D)
```

```python
import jax
import jax.numpy as jnp
import jax.experimental.pallas as pl
import jax.experimental.pallas.tpu as pltpu

B, SQ, D = 16, 80, 512
H, SK, DH = 32, 80, 128
M = B * SQ
TH = 8
NG = H // TH
NU = 2 * NG
CW = TH * DH
OCH = (560, 400, 240, 80)
OC = len(OCH)
OFF = tuple(sum(OCH[:i]) for i in range(OC + 1))
NQ = 4
FX = 240
FY = 240
FL = 320
KC = D // 128
bf = jnp.bfloat16
f32 = jnp.float32
NT = (((1,), (1,)), ((), ()))
SCALE = DH ** -0.5
SCOPES = False
LAST_Y = True

RAMP = ((320, 256), (480, 512), (800, 896), (M, CW))
S_XR = 0
S_WC = S_XR + len(RAMP)
S_XB = S_WC + len(RAMP)
S_WQ = S_XB + 1
S_K = S_WQ + NU
S_V = S_K + NU
S_WO = S_V + NU
S_N = S_WO + NU


class _Null:
    def __enter__(self):
        return self
    def __exit__(self, *a):
        return False


def _scope(name):
    return jax.named_scope(name) if SCOPES else _Null()


def _dot(a, b):
    return jnp.dot(a, b, preferred_element_type=f32)


def _chain(acc2, j, d):
    acc2[j % 2] = d if acc2[j % 2] is None else acc2[j % 2] + d


def _attention(get_q, get_k, get_v, x_op, x_done, y_op, fy):
    items = [(h, b) for h in range(TH) for b in range(B)]
    n = len(items)
    queues = {0: [], 1: [], 2: [], 3: []}
    for j in range(KC):
        queues[1 + 2 * (j % 2)].append(('X', j))
    for i in range(n):
        queues[2 * (i % 2)].append(('S', i))
        queues[1 + 2 * (i % 2)].append(('P', i))
    if y_op is not None:
        for j in range(KC):
            queues[2 * (j % 2)].append(('Y', j))
    cost = {'S': SQ, 'P': SQ, 'X': FX, 'Y': fy}
    load = [0, 0, 0, 0]
    res, soft, xs, ys = {}, {}, [None, None], [None, None]
    while any(queues.values()):
        cand = sorted(range(4), key=lambda m: (load[m], m))
        m = [c for c in cand if queues[c]][0]
        kind, idx = queues[m].pop(0)
        load[m] += cost[kind]
        if kind == 'S':
            h, b = items[idx]
            s = jax.lax.dot_general(get_q(h, b), get_k(h, b), NT, preferred_element_type=f32)
            p = jnp.exp(s - jnp.max(s, axis=-1, keepdims=True))
            soft[idx] = (p.astype(bf), jnp.sum(p, axis=-1, keepdims=True))
        elif kind == 'P':
            h, b = items[idx]
            p, l = soft.pop(idx)
            o = _dot(p, get_v(h, b))
            res[(h, b)] = (o * pl.reciprocal(l, approx=True)).astype(bf)
        elif kind == 'X':
            _chain(xs, idx, x_op(idx))
            if idx == KC - 1:
                x_done(xs)
        else:
            _chain(ys, idx, y_op(idx, res))
    o = jnp.concatenate(
        [jnp.concatenate([res[(h, b)] for b in range(B)], axis=0) for h in range(TH)], axis=1)
    return o, ys


def _body(xa, ka, va, wqa, woa, xb, kb, vb, wqb, wob, out_hbm,
          x_s, wq_s, wo_s, k_s, v_s, q_s, acc, stage, sem, sem_o):
    ks = (ka, kb); vs = (va, vb); wqs = (wqa, wqb); wos = (woa, wob)
    cp = pltpu.make_async_copy

    def x_cp(r0, nr, s):
        return cp(xa.at[pl.ds(r0, nr)], x_s.at[0, pl.ds(r0, nr)], sem.at[s])
    xr_cps, wc_cps = [], []
    pr = pc = 0
    for i, (r, c) in enumerate(RAMP):
        xr_cps.append(x_cp(pr, r - pr, S_XR + i) if r > pr else None)
        wc_cps.append(cp(wqa.at[:, pl.ds(pc, c - pc)], wq_s.at[0, :, pl.ds(pc, c - pc)], sem.at[S_WC + i]) if c > pc else None)
        pr, pc = r, c
    xb_cp = cp(xb, x_s.at[1], sem.at[S_XB])
    def wq_cp(u):
        br, g = divmod(u, NG)
        return cp(wqs[br].at[:, pl.ds(g * CW, CW)], wq_s.at[u], sem.at[S_WQ + u])
    def k_cp(u):
        br, g = divmod(u, NG)
        return cp(ks[br].at[:, pl.ds(g * TH, TH)], k_s.at[u], sem.at[S_K + u])
    def v_cp(u):
        br, g = divmod(u, NG)
        return cp(vs[br].at[:, pl.ds(g * TH, TH)], v_s.at[u], sem.at[S_V + u])
    def wo_cp(u):
        br, g = divmod(u, NG)
        return cp(wos[br].at[pl.ds(g * CW, CW)], wo_s.at[u], sem.at[S_WO + u])
    def wait_into(dst, s):
        cp(dst, dst, sem.at[s]).wait()
    outa_cp = cp(stage.at[0], out_hbm.at[:, pl.ds(0, D)], sem_o.at[OC])
    def outb_cp(c):
        return cp(stage.at[1, pl.ds(OFF[c], OCH[c])], out_hbm.at[pl.ds(OFF[c], OCH[c]), pl.ds(D, D)], sem_o.at[c])

    for wc, xr in zip(wc_cps, xr_cps):
        for c in (wc, xr):
            if c is not None:
                c.start()
    wq_cp(1).start()
    for u in range(NU):
        k_cp(u).start(); v_cp(u).start(); wo_cp(u).start()
        if u + 2 == NG:
            xb_cp.start()
        if u + 2 < NU:
            wq_cp(u + 2).start()

    def fin_q(q):
        return (q * SCALE).astype(bf)

    def fin_q2(v):
        return (v[0] * SCALE + v[1] * SCALE).astype(bf)

    def qproj(xv, w):
        return fin_q(_dot(xv, w))

    C7 = (TH - 1) * DH
    C6 = (TH - 2) * DH

    def attention(u, y_op, fy):
        br = u >> 2
        qslot = u & (NQ - 1)
        q7 = []
        def x_op(j):
            return _dot(x_s[br, 0:FX, j * 128:(j + 1) * 128], wq_s[u, j * 128:(j + 1) * 128, C7:CW])
        def x_done(v):
            q7.append(fin_q2(v))
        def get_q(h, b):
            if h == TH - 1 and (b + 1) * SQ <= FX:
                return q7[0][b * SQ:(b + 1) * SQ]
            return q_s[qslot, b * SQ:(b + 1) * SQ, h * DH:(h + 1) * DH]
        return _attention(get_q, lambda h, b: k_s[u, b, h], lambda h, b: v_s[u, b, h], x_op, x_done, y_op, fy)

    def q0_rect(r0, r1, c0, c1):
        if r0 >= r1 or c0 >= c1:
            return
        if c1 > C7 and r0 < FX:
            q0_rect(r0, r1, c0, C7)
            q0_rect(max(r0, FX), r1, max(c0, C7), c1)
            return
        q_s[0, r0:r1, c0:c1] = qproj(x_s[0, r0:r1, :], wq_s[0, :, c0:c1])
    pr = pc = 0
    for i, (r, c) in enumerate(RAMP):
        with _scope("R%d" % i):
            for d in (wc_cps[i], xr_cps[i]):
                if d is not None:
                    d.wait()
            if i == len(RAMP) - 1:
                wq_cp(1).wait()
            q0_rect(pr, r, 0, pc)
            q0_rect(0, r, pc, c)
            if i == len(RAMP) - 1:
                q_s[1, :, 0:C7] = qproj(x_s[0], wq_s[1, :, 0:C7])
                q_s[1, FX:M, C7:CW] = qproj(x_s[0, FX:M, :], wq_s[1, :, C7:CW])
        pr, pc = r, c

    def step(u, carry):
        with _scope("step"):
            br = u >> 2
            un = u + 2
            bn = un >> 2
            ns = un & (NQ - 1)
            wait_into(k_s.at[u], S_K + u)
            wait_into(v_s.at[u], S_V + u)
            wait_into(wo_s.at[u], S_WO + u)
            wait_into(wq_s.at[un], S_WQ + un)
            @pl.when(un == NG)
            def _():
                xb_cp.wait()
            def y_op(j, res):
                return _dot(x_s[bn, 0:FY, j * 128:(j + 1) * 128], wq_s[un, j * 128:(j + 1) * 128, C6:C7])
            o, qy = attention(u, y_op, FY)
            q_s[ns, 0:FY, C6:C7] = fin_q2(qy)
            q_s[ns, :, 0:C6] = qproj(x_s[bn], wq_s[un, :, 0:C6])
            if FX == FY:
                q_s[ns, FX:M, C6:CW] = qproj(x_s[bn, FX:M, :], wq_s[un, :, C6:CW])
            else:
                q_s[ns, FY:M, C6:C7] = qproj(x_s[bn, FY:M, :], wq_s[un, :, C6:C7])
                q_s[ns, FX:M, C7:CW] = qproj(x_s[bn, FX:M, :], wq_s[un, :, C7:CW])
            prev = jnp.where((u & (NG - 1)) == 0, 0.0, acc[br])
            t = prev + _dot(o, wo_s[u])
            acc[br] = t
            stage[br] = t.astype(bf)
            @pl.when(u == NG - 1)
            def _():
                outa_cp.start()
        return carry
    jax.lax.fori_loop(0, NU - 2, step, 0)

    def last(u, carry):
        with _scope("last"):
            wait_into(k_s.at[u], S_K + u)
            wait_into(v_s.at[u], S_V + u)
            wait_into(wo_s.at[u], S_WO + u)
            def y_op(j, res):
                lhs = jnp.concatenate([res[(j, b)] for b in range(FL // SQ)], axis=0)
                return _dot(lhs, wo_s[u, j * 128:(j + 1) * 128, 0:128])
            o, oy = attention(u, y_op if LAST_Y else None, FL)
            for c in range(OC):
                r0, r1 = OFF[c], OFF[c + 1]
                if c == 0 and LAST_Y:
                    ta = (acc[1, 0:FL, 0:128] + oy[0]) + (oy[1] + _dot(o[0:FL, KC * 128:], wo_s[u, KC * 128:, 0:128]))
                    tb = _dot(o[0:FL], wo_s[u, :, 128:D])
                    tc = _dot(o[FL:r1], wo_s[u])
                    tb = acc[1, 0:FL, 128:D] + tb
                    tc = acc[1, FL:r1, :] + tc
                    t = jnp.concatenate([jnp.concatenate([ta, tb], axis=1), tc], axis=0)
                else:
                    t = acc[1, r0:r1, :] + _dot(o[r0:r1], wo_s[u])
                acc[1, r0:r1, :] = t
                stage[1, r0:r1, :] = t.astype(bf)
                @pl.when(u == NU - 1)
                def _():
                    outb_cp(c).start()
        return carry
    jax.lax.fori_loop(NU - 2, NU, last, 0)
    with _scope("tail"):
        outa_cp.wait()
        for c in range(OC):
            outb_cp(c).wait()


@jax.jit
def pallas_concat_heads__mha_block_cached__mha_block_cached__near_ridge_kernel(
    A_x, A_k_cache, A_v_cache, A_wq, A_wo, B_x, B_k_cache, B_v_cache, B_wq, B_wo):
    xa = A_x.reshape(M, D)
    xb = B_x.reshape(M, D)
    any_spec = pl.BlockSpec(memory_space=pl.ANY)
    DMA = pltpu.SemaphoreType.DMA
    out = pl.pallas_call(
        _body,
        in_specs=[any_spec] * 10,
        out_specs=any_spec,
        out_shape=jax.ShapeDtypeStruct((M, 2 * D), bf),
        scratch_shapes=[
            pltpu.VMEM((2, M, D), bf),
            pltpu.VMEM((NU, D, CW), bf),
            pltpu.VMEM((NU, CW, D), bf),
            pltpu.VMEM((NU, B, TH, SK, DH), bf),
            pltpu.VMEM((NU, B, TH, SK, DH), bf),
            pltpu.VMEM((NQ, M, CW), bf),
            pltpu.VMEM((2, M, D), f32),
            pltpu.VMEM((2, M, D), bf),
            DMA((S_N,)), DMA((OC + 1,)),
        ],
        compiler_params=pltpu.CompilerParams(vmem_limit_bytes=120 * 1024 * 1024,
                                             disable_semaphore_checks=True),
    )(xa, A_k_cache, A_v_cache, A_wq, A_wo, xb, B_k_cache, B_v_cache, B_wq, B_wo)
    return out.reshape(B, SQ, 2 * D)
```

```python
import jax
import jax.numpy as jnp
import jax.experimental.pallas as pl
import jax.experimental.pallas.tpu as pltpu

B, SQ, D = 16, 80, 512
H, SK, DH = 32, 80, 128
M = B * SQ
TH = 8
NG = H // TH
NU = 2 * NG
CW = TH * DH
KC = D // 128
C6 = (TH - 2) * DH
C7 = (TH - 1) * DH
NQ = 4
FX = 240
FL = 320
RAMP = ((320, 256), (480, 512), (800, 896), (M, CW))
OCH = (560, 400, 240, 80)
OFF = tuple(sum(OCH[:i]) for i in range(len(OCH) + 1))

S_XR = 0
S_WC = S_XR + len(RAMP)
S_XB = S_WC + len(RAMP)
S_WQ = S_XB + 1
S_K = S_WQ + NU
S_V = S_K + NU
S_WO = S_V + NU
S_N = S_WO + NU

bf16 = jnp.bfloat16
f32 = jnp.float32
SCALE = DH ** -0.5


def _dot(a, b):
    return jnp.dot(a, b, preferred_element_type=f32)


def _attention(get_q, get_k, get_v, x_op, x_done, y_op, fy):
    items = [(h, b) for h in range(TH) for b in range(B)]
    queues = [[], [], [], []]
    for j in range(KC):
        queues[1 + 2 * (j % 2)].append(('X', j))
    for i in range(len(items)):
        queues[2 * (i % 2)].append(('S', i))
        queues[1 + 2 * (i % 2)].append(('P', i))
    for j in range(KC):
        queues[2 * (j % 2)].append(('Y', j))
    cost = {'S': SQ, 'P': SQ, 'X': FX, 'Y': fy}
    load = [0, 0, 0, 0]
    res, soft, xs, ys = {}, {}, [None, None], [None, None]

    def chain(acc2, j, d):
        acc2[j % 2] = d if acc2[j % 2] is None else acc2[j % 2] + d

    while any(queues):
        m = min((c for c in range(4) if queues[c]), key=lambda c: (load[c], c))
        kind, idx = queues[m].pop(0)
        load[m] += cost[kind]
        if kind == 'S':
            h, b = items[idx]
            s = jax.lax.dot_general(get_q(h, b), get_k(h, b), (((1,), (1,)), ((), ())),
                                    preferred_element_type=f32)
            p = jnp.exp(s - jnp.max(s, axis=-1, keepdims=True))
            soft[idx] = (p.astype(bf16), jnp.sum(p, axis=-1, keepdims=True))
        elif kind == 'P':
            h, b = items[idx]
            p, l = soft.pop(idx)
            o = _dot(p, get_v(h, b))
            res[(h, b)] = (o * pl.reciprocal(l, approx=True)).astype(bf16)
        elif kind == 'X':
            chain(xs, idx, x_op(idx))
            if idx == KC - 1:
                x_done(xs)
        else:
            chain(ys, idx, y_op(idx, res))
    o = jnp.concatenate(
        [jnp.concatenate([res[(h, b)] for b in range(B)], axis=0) for h in range(TH)], axis=1)
    return o, ys


def _body(xa, ka, va, wqa, woa, xb, kb, vb, wqb, wob, out_hbm,
          x_s, wq_s, wo_s, k_s, v_s, q_s, acc, stage, sem, sem_o):
    copy = pltpu.make_async_copy
    ks, vs, wqs, wos = (ka, kb), (va, vb), (wqa, wqb), (woa, wob)

    ramp_cps = []
    pr = pc = 0
    for i, (r, c) in enumerate(RAMP):
        ramp_cps.append([
            copy(wqa.at[:, pl.ds(pc, c - pc)], wq_s.at[0, :, pl.ds(pc, c - pc)], sem.at[S_WC + i]),
            copy(xa.at[pl.ds(pr, r - pr)], x_s.at[0, pl.ds(pr, r - pr)], sem.at[S_XR + i]),
        ])
        pr, pc = r, c
    xb_cp = copy(xb, x_s.at[1], sem.at[S_XB])

    def wq_cp(u):
        br, g = divmod(u, NG)
        return copy(wqs[br].at[:, pl.ds(g * CW, CW)], wq_s.at[u], sem.at[S_WQ + u])

    def k_cp(u):
        br, g = divmod(u, NG)
        return copy(ks[br].at[:, pl.ds(g * TH, TH)], k_s.at[u], sem.at[S_K + u])

    def v_cp(u):
        br, g = divmod(u, NG)
        return copy(vs[br].at[:, pl.ds(g * TH, TH)], v_s.at[u], sem.at[S_V + u])

    def wo_cp(u):
        br, g = divmod(u, NG)
        return copy(wos[br].at[pl.ds(g * CW, CW)], wo_s.at[u], sem.at[S_WO + u])

    def wait_filled(dst, s):
        copy(dst, dst, sem.at[s]).wait()

    outa_cp = copy(stage.at[0], out_hbm.at[:, pl.ds(0, D)], sem_o.at[len(OCH)])

    def outb_cp(c):
        return copy(stage.at[1, pl.ds(OFF[c], OCH[c])],
                    out_hbm.at[pl.ds(OFF[c], OCH[c]), pl.ds(D, D)], sem_o.at[c])

    for cps in ramp_cps:
        for c in cps:
            c.start()
    wq_cp(1).start()
    for u in range(NU):
        k_cp(u).start()
        v_cp(u).start()
        wo_cp(u).start()
        if u + 2 == NG:
            xb_cp.start()
        if u + 2 < NU:
            wq_cp(u + 2).start()

    def qproj(xv, w):
        return (_dot(xv, w) * SCALE).astype(bf16)

    def q_of_chains(v):
        return (v[0] * SCALE + v[1] * SCALE).astype(bf16)

    def attention(u, y_op, fy):
        br = u >> 2
        slot = u & (NQ - 1)
        q7 = []

        def x_op(j):
            return _dot(x_s[br, 0:FX, j * 128:(j + 1) * 128],
                        wq_s[u, j * 128:(j + 1) * 128, C7:CW])

        def get_q(h, b):
            if h == TH - 1 and (b + 1) * SQ <= FX:
                return q7[0][b * SQ:(b + 1) * SQ]
            return q_s[slot, b * SQ:(b + 1) * SQ, h * DH:(h + 1) * DH]

        return _attention(get_q, lambda h, b: k_s[u, b, h], lambda h, b: v_s[u, b, h],
                          x_op, lambda v: q7.append(q_of_chains(v)), y_op, fy)

    def q0_rect(r0, r1, c0, c1):
        if r0 >= r1 or c0 >= c1:
            return
        if c1 > C7 and r0 < FX:
            q0_rect(r0, r1, c0, C7)
            q0_rect(FX, r1, max(c0, C7), c1)
            return
        q_s[0, r0:r1, c0:c1] = qproj(x_s[0, r0:r1, :], wq_s[0, :, c0:c1])

    pr = pc = 0
    for i, (r, c) in enumerate(RAMP):
        for d in ramp_cps[i]:
            d.wait()
        if i == len(RAMP) - 1:
            wq_cp(1).wait()
        q0_rect(pr, r, 0, pc)
        q0_rect(0, r, pc, c)
        pr, pc = r, c
    q_s[1, :, 0:C7] = qproj(x_s[0], wq_s[1, :, 0:C7])
    q_s[1, FX:M, C7:CW] = qproj(x_s[0, FX:M, :], wq_s[1, :, C7:CW])

    def step(u, carry):
        br = u >> 2
        un = jnp.minimum(u + 2, NU - 1)
        bn = un >> 2
        ns = un & (NQ - 1)
        wait_filled(k_s.at[u], S_K + u)
        wait_filled(v_s.at[u], S_V + u)
        wait_filled(wo_s.at[u], S_WO + u)
        wait_filled(wq_s.at[un], S_WQ + un)

        @pl.when(un == NG)
        def _():
            xb_cp.wait()

        def y_op(j, res):
            return _dot(x_s[bn, 0:FX, j * 128:(j + 1) * 128],
                        wq_s[un, j * 128:(j + 1) * 128, C6:C7])

        o, qy = attention(u, y_op, FX)
        q_s[ns, 0:FX, C6:C7] = q_of_chains(qy)
        q_s[ns, :, 0:C6] = qproj(x_s[bn], wq_s[un, :, 0:C6])
        q_s[ns, FX:M, C6:CW] = qproj(x_s[bn, FX:M, :], wq_s[un, :, C6:CW])
        prev = jnp.where((u & (NG - 1)) == 0, 0.0, acc[br])
        t = prev + _dot(o, wo_s[u])
        acc[br] = t
        stage[br] = t.astype(bf16)

        @pl.when(u == NG - 1)
        def _():
            outa_cp.start()
        return carry

    def last(u, carry):
        wait_filled(k_s.at[u], S_K + u)
        wait_filled(v_s.at[u], S_V + u)
        wait_filled(wo_s.at[u], S_WO + u)

        def y_op(j, res):
            lhs = jnp.concatenate([res[(j, b)] for b in range(FL // SQ)], axis=0)
            return _dot(lhs, wo_s[u, j * 128:(j + 1) * 128, 0:128])

        o, oy = attention(u, y_op, FL)
        for c in range(len(OCH)):
            r0, r1 = OFF[c], OFF[c + 1]
            if c == 0:
                ta = (acc[1, 0:FL, 0:128] + oy[0]) + (
                    oy[1] + _dot(o[0:FL, KC * 128:], wo_s[u, KC * 128:, 0:128]))
                tb = acc[1, 0:FL, 128:D] + _dot(o[0:FL], wo_s[u, :, 128:D])
                tc = acc[1, FL:r1, :] + _dot(o[FL:r1], wo_s[u])
                t = jnp.concatenate([jnp.concatenate([ta, tb], axis=1), tc], axis=0)
            else:
                t = acc[1, r0:r1, :] + _dot(o[r0:r1], wo_s[u])
            acc[1, r0:r1, :] = t
            stage[1, r0:r1, :] = t.astype(bf16)

            @pl.when(u == NU - 1)
            def _():
                outb_cp(c).start()
        return carry

    def unit(u, carry):
        @pl.when(u < NU - 2)
        def _():
            step(u, carry)

        @pl.when(u >= NU - 2)
        def _():
            last(u, carry)
        return carry

    jax.lax.fori_loop(0, NU, unit, 0)
    outa_cp.wait()
    for c in range(len(OCH)):
        outb_cp(c).wait()


@jax.jit
def pallas_concat_heads__mha_block_cached__mha_block_cached__near_ridge_kernel(
    A_x: jax.Array,
    A_k_cache: jax.Array,
    A_v_cache: jax.Array,
    A_wq: jax.Array,
    A_wo: jax.Array,
    B_x: jax.Array,
    B_k_cache: jax.Array,
    B_v_cache: jax.Array,
    B_wq: jax.Array,
    B_wo: jax.Array,
):
    hbm = pl.BlockSpec(memory_space=pl.ANY)
    out = pl.pallas_call(
        _body,
        in_specs=[hbm] * 10,
        out_specs=hbm,
        out_shape=jax.ShapeDtypeStruct((M, 2 * D), bf16),
        scratch_shapes=[
            pltpu.VMEM((2, M, D), bf16),
            pltpu.VMEM((NU, D, CW), bf16),
            pltpu.VMEM((NU, CW, D), bf16),
            pltpu.VMEM((NU, B, TH, SK, DH), bf16),
            pltpu.VMEM((NU, B, TH, SK, DH), bf16),
            pltpu.VMEM((NQ, M, CW), bf16),
            pltpu.VMEM((2, M, D), f32),
            pltpu.VMEM((2, M, D), bf16),
            pltpu.SemaphoreType.DMA((S_N,)),
            pltpu.SemaphoreType.DMA((len(OCH) + 1,)),
        ],
        compiler_params=pltpu.CompilerParams(
            vmem_limit_bytes=120 * 1024 * 1024,
            disable_semaphore_checks=True),
    )(A_x.reshape(M, D), A_k_cache, A_v_cache, A_wq, A_wo,
      B_x.reshape(M, D), B_k_cache, B_v_cache, B_wq, B_wo)
    return out.reshape(B, SQ, 2 * D)
```
